```python
import os as _os
_os.environ.setdefault("JAX_PLATFORMS", "cpu")
import jax
import jax.numpy as jnp

def _softmax(x, axis=-1):
    return jax.nn.softmax(x, axis=axis)
def _gelu(x):
    return jax.nn.gelu(x, approximate=True)
def _silu(x):
    return jax.nn.silu(x)
def _sigmoid(x):
    return jax.nn.sigmoid(x)
def _layernorm(x, axis=-1, eps=1e-5):
    m = jnp.mean(x, axis=axis, keepdims=True)
    v = jnp.var(x, axis=axis, keepdims=True)
    return (x - m) / jnp.sqrt(v + eps)
def _scatter_add(tgt, idx, src, axis=0):
    return tgt.at[idx].add(src)
def _segment_sum(src, seg, n):
    return jax.ops.segment_sum(src, seg, n)
class _Rng:
    def __init__(self, key):
        self._k = key
    def _next(self):
        self._k, sub = jax.random.split(self._k)
        return sub
    def normal(self, shape):
        return jax.random.normal(self._next(), shape, dtype=jnp.bfloat16)
    def randint(self, lo, hi, shape):
        return jax.random.randint(self._next(), shape, lo, hi, dtype=jnp.int32)
    def uniform(self, shape, lo=0.0, hi=1.0):
        return jax.random.uniform(self._next(), shape, jnp.bfloat16, lo, hi)
    def permutation(self, n):
        return jax.random.permutation(self._next(), n)


kernel_name = 'standalone__grn__sampling'

def setup_inputs():
    _rng = _Rng(jax.random.key(int.from_bytes(__import__("os").urandom(4), "little")))
    _w = (lambda a: (lambda t: t.astype(jnp.bfloat16) if jnp.issubdtype(t.dtype, jnp.floating) else t)(jnp.asarray(a)))
    B, S, D = 512, 32, 640
    return {
        "x": _w((lambda *s: _rng.normal(s) * 0.05)(B, S, D)),
        "g": _w((lambda *s: _rng.normal(s) * 0.1)(D) * 0.1),
        "b": _w((lambda *s: _rng.normal(s) * 0.1)(D) * 0.1),
    }

def reference(x, g, b):
    gx = jnp.sqrt((x * x).sum(axis=-2, keepdims=True))
    nx = gx / (gx.mean(axis=-1, keepdims=True) + 1e-6)
    return g * (x * nx) + b + x
```

```python
import jax
import jax.numpy as jnp
from jax import lax
import jax.experimental.pallas as pl
import jax.experimental.pallas.tpu as pltpu

WAYS = 8
HEAD = 4
TAIL = 1
EPS = 1e-6


def _grn_slab(buf, j, g, b):
    ways, _, _, d = buf.shape
    sumsq = []
    for w in range(ways):
        x = buf[w, j].astype(jnp.float32)
        sumsq.append(jnp.sum(x * x, axis=0, keepdims=True))
    gx = jnp.sqrt(jnp.concatenate(sumsq, axis=0))
    mean = jnp.sum(gx, axis=-1, keepdims=True) / d
    scale = g * (gx / (mean + EPS)) + 1.0
    for w in range(ways):
        x = buf[w, j].astype(jnp.float32)
        buf[w, j] = (x * scale[w:w + 1] + b).astype(buf.dtype)


def _grn_kernel(x_hbm, g_hbm, b_hbm, o_hbm, buf, g_vmem, b_vmem, sems):
    _, n, _, d = buf.shape
    bounds = (0, HEAD, n - TAIL, n)
    reads = [
        pltpu.make_async_copy(x_hbm.at[:, lo:hi], buf.at[:, lo:hi], sems.at[k])
        for k, (lo, hi) in enumerate(zip(bounds[:-1], bounds[1:]))
    ]
    read_g = pltpu.make_async_copy(g_hbm, g_vmem, sems.at[3])
    read_b = pltpu.make_async_copy(b_hbm, b_vmem, sems.at[3])

    def write(j):
        pltpu.make_async_copy(
            buf.at[:, pl.ds(j, 1)], o_hbm.at[:, pl.ds(j, 1)], sems.at[4]
        ).start()

    reads[0].start()
    read_g.start()
    read_b.start()
    reads[1].start()
    reads[2].start()

    read_g.wait()
    read_b.wait()
    g = g_vmem[...].astype(jnp.float32).reshape(1, d)
    b = b_vmem[...].astype(jnp.float32).reshape(1, d)

    def compute(j, carry):
        _grn_slab(buf, j, g, b)
        return carry

    def compute_and_write(j, carry):
        _grn_slab(buf, j, g, b)
        write(j)
        return carry

    reads[0].wait()
    lax.fori_loop(0, HEAD, compute, 0)
    reads[1].wait()
    for j in range(HEAD):
        write(j)
    lax.fori_loop(HEAD, n - TAIL, compute_and_write, 0)
    reads[2].wait()
    lax.fori_loop(n - TAIL, n, compute_and_write, 0)
    pltpu.make_async_copy(buf, o_hbm, sems.at[4]).wait()


@jax.jit
def pallas_standalone__grn__sampling_kernel(
    x: jax.Array,
    g: jax.Array,
    b: jax.Array,
):
    batch, s, d = x.shape
    shape = (WAYS, batch // WAYS, s, d)
    hbm = pl.BlockSpec(memory_space=pltpu.HBM)
    out = pl.pallas_call(
        _grn_kernel,
        in_specs=[hbm, hbm, hbm],
        out_specs=hbm,
        out_shape=jax.ShapeDtypeStruct(shape, x.dtype),
        scratch_shapes=[
            pltpu.VMEM(shape, x.dtype),
            pltpu.VMEM((d,), g.dtype),
            pltpu.VMEM((d,), b.dtype),
            pltpu.SemaphoreType.DMA((5,)),
        ],
        compiler_params=pltpu.CompilerParams(vmem_limit_bytes=64 * 1024 * 1024),
    )(x.reshape(shape), g, b)
    return out.reshape(batch, s, d)
```

```python
import jax
import jax.numpy as jnp
from jax import lax
import jax.experimental.pallas as pl
import jax.experimental.pallas.tpu as pltpu

EPS = 1e-6
STREAM_BYTES = 2 * 1024 * 1024
WAYS = 5
READ_SPLIT = 2
STEP_ROWS = 3
HEAD_STEPS = 6
LOOKAHEAD_ROWS = 6
TAIL_ROWS = 2


def _grn_in_place(ref, items, g, b):
    sumsq = []
    for item in items:
        x = ref[item].astype(jnp.float32)
        sumsq.append(jnp.sum(x * x, axis=0, keepdims=True))
    gx = jnp.sqrt(jnp.concatenate(sumsq, axis=0))
    mean = jnp.sum(gx, axis=-1, keepdims=True) / gx.shape[-1]
    scale = g * (gx / (mean + EPS)) + 1.0
    for k, item in enumerate(items):
        x = ref[item].astype(jnp.float32)
        ref[item] = (x * scale[k:k + 1] + b).astype(ref.dtype)


def _loop(lo, hi, body):
    lax.fori_loop(lo, hi, lambda i, carry: body(i), None)


def _grn_kernel(x_hbm, g_hbm, b_hbm, o_hbm, buf, rest, g_vmem, b_vmem, out_sem):
    streams, rows, s, d = buf.shape
    tiled = streams * rows
    steps_per_group = rows // STEP_ROWS
    head_rows = HEAD_STEPS * STEP_ROWS
    body_rows = rows - TAIL_ROWS
    piece = s // READ_SPLIT

    def affine():
        g = g_vmem[...].astype(jnp.float32).reshape(1, d)
        b = b_vmem[...].astype(jnp.float32).reshape(1, d)
        return g, b

    def row_items(w0, j):
        return [(w0 + w, j) for w in range(WAYS)]

    def step_items(w0, j0):
        return [it for k in range(STEP_ROWS) for it in row_items(w0, j0 + k)]

    def write(items):
        for w, j in items:
            pltpu.make_async_copy(
                buf.at[w, j], o_hbm.at[w * rows + j], out_sem
            ).start()

    def read_phase(small_sem, head_sem, body_sem, tail_sem):
        def read_rows(lo, hi, sem):
            def read_row(j):
                for r in range(0, s, piece):
                    for w in range(streams):
                        pltpu.make_async_copy(
                            x_hbm.at[w * rows + j, pl.ds(r, piece)],
                            buf.at[w, j, pl.ds(r, piece)],
                            sem,
                        ).start(priority=w % 2)

            _loop(lo, hi, read_row)

        def wait_rows(lo, hi, sem):
            filled = buf.at[:, lo:hi]
            pltpu.make_async_copy(filled, filled, sem).wait()

        small = [
            pltpu.make_async_copy(g_hbm, g_vmem, small_sem),
            pltpu.make_async_copy(b_hbm, b_vmem, small_sem),
            pltpu.make_async_copy(x_hbm.at[tiled:], rest, small_sem),
        ]
        queued = head_rows + LOOKAHEAD_ROWS
        read_rows(0, head_rows, head_sem)
        for copy in small:
            copy.start()
        read_rows(head_rows, queued, body_sem)

        wait_rows(0, head_rows, head_sem)
        for copy in small:
            copy.wait()
        g, b = affine()
        _grn_in_place(rest, range(rest.shape[0]), g, b)

        def head_step(q):
            j0 = q * STEP_ROWS
            read_rows(queued + j0, queued + j0 + STEP_ROWS, body_sem)
            _grn_in_place(buf, step_items(0, j0), g, b)

        _loop(0, HEAD_STEPS, head_step)
        read_rows(queued + head_rows, body_rows, body_sem)
        read_rows(body_rows, rows, tail_sem)

        wait_rows(head_rows, body_rows, body_sem)
        _loop(0, head_rows, lambda j: write(row_items(0, j)))
        wait_rows(body_rows, rows, tail_sem)

    pl.run_scoped(read_phase, *[pltpu.SemaphoreType.DMA(())] * 4)

    g, b = affine()

    def step(q):
        w0 = lax.div(q, steps_per_group) * WAYS
        j0 = lax.rem(q, steps_per_group) * STEP_ROWS
        items = step_items(w0, j0)
        _grn_in_place(buf, items, g, b)
        write(items)

    _loop(HEAD_STEPS, streams // WAYS * steps_per_group, step)
    pltpu.make_async_copy(rest, o_hbm.at[tiled:], out_sem).start()
    pltpu.make_async_copy(o_hbm, o_hbm, out_sem).wait()


@jax.jit
def pallas_standalone__grn__sampling_kernel(
    x: jax.Array,
    g: jax.Array,
    b: jax.Array,
):
    batch, s, d = x.shape
    rows = STREAM_BYTES // (s * d * x.dtype.itemsize) // STEP_ROWS * STEP_ROWS
    streams = (batch - 1) // (rows * WAYS) * WAYS
    assert streams > 0
    assert 2 * HEAD_STEPS * STEP_ROWS + LOOKAHEAD_ROWS + TAIL_ROWS <= rows

    hbm = pl.BlockSpec(memory_space=pltpu.HBM)
    return pl.pallas_call(
        _grn_kernel,
        in_specs=[hbm, hbm, hbm],
        out_specs=hbm,
        out_shape=jax.ShapeDtypeStruct(x.shape, x.dtype),
        scratch_shapes=[
            pltpu.VMEM((streams, rows, s, d), x.dtype),
            pltpu.VMEM((batch - streams * rows, s, d), x.dtype),
            pltpu.VMEM((d,), g.dtype),
            pltpu.VMEM((d,), b.dtype),
            pltpu.SemaphoreType.DMA(()),
        ],
        compiler_params=pltpu.CompilerParams(vmem_limit_bytes=32 * 1024 * 1024),
    )(x, g, b)
```
